```python
import os as _os
_os.environ.setdefault("JAX_PLATFORMS", "cpu")
import jax
import jax.numpy as jnp

def _softmax(x, axis=-1):
    return jax.nn.softmax(x, axis=axis)
def _gelu(x):
    return jax.nn.gelu(x, approximate=True)
def _silu(x):
    return jax.nn.silu(x)
def _sigmoid(x):
    return jax.nn.sigmoid(x)
def _layernorm(x, axis=-1, eps=1e-5):
    m = jnp.mean(x, axis=axis, keepdims=True)
    v = jnp.var(x, axis=axis, keepdims=True)
    return (x - m) / jnp.sqrt(v + eps)
def _scatter_add(tgt, idx, src, axis=0):
    return tgt.at[idx].add(src)
def _segment_sum(src, seg, n):
    return jax.ops.segment_sum(src, seg, n)
class _Rng:
    def __init__(self, key):
        self._k = key
    def _next(self):
        self._k, sub = jax.random.split(self._k)
        return sub
    def normal(self, shape):
        return jax.random.normal(self._next(), shape, dtype=jnp.bfloat16)
    def randint(self, lo, hi, shape):
        return jax.random.randint(self._next(), shape, lo, hi, dtype=jnp.int32)
    def uniform(self, shape, lo=0.0, hi=1.0):
        return jax.random.uniform(self._next(), shape, jnp.bfloat16, lo, hi)
    def permutation(self, n):
        return jax.random.permutation(self._next(), n)


kernel_name = 'sequential_preLN__softmax_full_mha__dense_activation_squared_relu__prompt'

def setup_inputs():
    _rng = _Rng(jax.random.key(int.from_bytes(__import__("os").urandom(4), "little")))
    _w = (lambda a: (lambda t: t.astype(jnp.bfloat16) if jnp.issubdtype(t.dtype, jnp.floating) else t)(jnp.asarray(a)))
    def _A_setup():
        B, S, D = 1, 2048, 448
        return {
            "x": _w((lambda *s: _rng.normal(s) * 0.05)(B, S, D)),
            "wqkv": _w((lambda *s: _rng.normal(s) * 0.05)(D, 3 * D)),
            "wo": _w((lambda *s: _rng.normal(s) * 0.05)(D, D)),
        }
    _A_in = _A_setup()

    def _B_setup():
        B, S, D, F = 1, 2048, 448, 1792
        return {
            "x": _w((lambda *s: _rng.normal(s) * 0.05)(B, S, D)),
            "w1": _w((lambda *s: _rng.normal(s) * 0.05)(D, F)),
            "b1": _w((lambda *s: _rng.normal(s) * 0.05)(F)),
            "w2": _w((lambda *s: _rng.normal(s) * 0.05)(F, D)),
            "b2": _w((lambda *s: _rng.normal(s) * 0.05)(D)),
        }
    _B_in = _B_setup()

    return {
        "A_x": _A_in["x"],
        "A_wqkv": _A_in["wqkv"],
        "A_wo": _A_in["wo"],
        "B_x": _B_in["x"],
        "B_w1": _B_in["w1"],
        "B_b1": _B_in["b1"],
        "B_w2": _B_in["w2"],
        "B_b2": _B_in["b2"],
    }

def reference(A_x, A_wqkv, A_wo, B_x, B_w1, B_b1, B_w2, B_b2):
    def _A_ref(x, wqkv, wo):
        B, S, D = x.shape
        H = 16; Dh = D // H
        qkv = (lambda x, *d: x.transpose(*d))((x @ wqkv).reshape(B, S, 3, H, Dh), 2, 0, 3, 1, 4)
        q, k, v = qkv[0], qkv[1], qkv[2]
        scale = Dh ** -0.5
        scores = jnp.einsum("bhqd,bhkd->bhqk", q, k) * scale
        p = _softmax(scores, axis=-1)
        o = jnp.einsum("bhqk,bhkd->bhqd", p, v)
        return (lambda x, *d: x.transpose(*d))(o, 0, 2, 1, 3).reshape(B, S, D) @ wo

    def _B_ref(x, w1, b1, w2, b2):
        h = jnp.einsum("bsd,df->bsf", x, w1) + b1
        zero = jnp.zeros_like(h)
        r = jnp.where(h > zero, h, zero)
        h = r * r
        out = jnp.einsum("bsf,fd->bsd", h, w2) + b2
        return out

    x = A_x
    h = x + _A_ref(_layernorm(x, axis=-1), A_wqkv, A_wo)
    h2 = h + _B_ref(_layernorm(h, axis=-1), B_w1, B_b1, B_w2, B_b2)
    return h2
```

```python
import functools
import math

import jax
import jax.numpy as jnp
from jax import lax
import jax.experimental.pallas as pl
import jax.experimental.pallas.tpu as pltpu

S, D, H, F = 2048, 448, 16, 1792
DH = D // H
HP = 32
G = 4
GW = G * DH
KP = 512
BQ = 512
CK = 128
NC = S // CK
NQ = S // BQ
EPS = 1e-5
QSCALE = DH ** -0.5 * math.log2(math.e)

f32, bf16 = jnp.float32, jnp.bfloat16


def _dot(a, b):
    return jnp.dot(a, b, preferred_element_type=f32)


def _layernorm_t(x):
    mean = jnp.sum(x, axis=0, keepdims=True) * (1.0 / D)
    xc = x - mean
    var = jnp.sum(xc * xc, axis=0, keepdims=True) * (1.0 / D)
    return xc * lax.rsqrt(var + EPS)


def _head_rows(a, h, fill):
    row = lax.broadcasted_iota(jnp.int32, (HP, a.shape[1]), 0)
    if h % 2 == 0:
        return jnp.where(row < DH, a[DH * h:DH * h + HP], fill)
    return jnp.where(row >= HP - DH, a[DH * (h + 1) - HP:DH * (h + 1)], fill)


def _kernel(LAG, TN0, TN2,
            xt_hbm, wqkv_hbm, wo_hbm, w1_hbm, b1_ref, w2t_hbm, b2_ref, out_hbm,
            xt, wqkv, wo, w1, w2t, wqkvt, wot, w1t, b2c, qt, kk, vt, ot, yt,
            s0, s1, s2, s3, sem_x, sem_w, sem_o):
    sbuf = (s0, s1, s2, s3)

    n0 = S // TN0
    x_cp = [pltpu.make_async_copy(xt_hbm.at[:, pl.ds(c * TN0, TN0)],
                                  xt.at[:, pl.ds(c * TN0, TN0)], sem_x.at[c]) for c in range(n0)]
    w_cp = [pltpu.make_async_copy(src, dst, sem_w.at[i]) for i, (src, dst) in enumerate(
        ((wqkv_hbm, wqkv), (wo_hbm, wo), (w1_hbm, w1), (w2t_hbm, w2t)))]
    w_cp[0].start()
    for cp in x_cp:
        cp.start()
    for cp in w_cp[1:]:
        cp.start()

    w_cp[0].wait()
    wqkvt[...] = wqkv[...].T

    x_cp[0].wait()
    ln = _layernorm_t(xt[:, pl.ds(0, TN0)].astype(f32)).astype(bf16)
    for c in range(n0):
        cols = pl.ds(c * TN0, TN0)
        cur = ln
        if c + 1 < n0:
            x_cp[c + 1].wait()
            ln = _layernorm_t(xt[:, pl.ds((c + 1) * TN0, TN0)].astype(f32)).astype(bf16)
        k = _dot(wqkvt[pl.ds(D, D), :], cur).astype(bf16)
        zpad = jnp.zeros((128 - GW, TN0), bf16)
        for g in range(H // G):
            kk[g, cols, :] = jnp.concatenate([k[GW * g:GW * (g + 1)], zpad], axis=0).T
        qt[:, cols] = (_dot(wqkvt[pl.ds(0, D), :], cur) * QSCALE).astype(bf16)
        v = _dot(wqkvt[pl.ds(2 * D, D), :], cur)
        for h in range(H):
            vt[h, :, cols] = _head_rows(v, h, 1.0).astype(bf16)

    for cp in w_cp[1:]:
        cp.wait()
    wo32 = wo[...].astype(f32)
    wot[...] = jnp.concatenate([_head_rows(wo32, h, 0.0) for h in range(H)], axis=0).astype(bf16).T
    row = lax.broadcasted_iota(jnp.int32, (KP - D, F), 0)
    b1_rows = jnp.where(row == 0, b1_ref[...].astype(f32), 0.0).astype(bf16)
    w1t[...] = jnp.concatenate([w1[...], b1_rows], axis=0).T
    b2c[...] = jnp.broadcast_to(b2_ref[...].astype(f32), (128, D)).T

    def load_q(g, qb, j):
        lo, hi = (DH * j) // 16 * 16, -(-(DH * (j + 1)) // 16) * 16
        q = qt[pl.ds(pl.multiple_of(g * GW + lo, 16), hi - lo), pl.ds(pl.multiple_of(qb * BQ, BQ), BQ)]
        q = pltpu.bitcast(q, jnp.uint32)
        r = lax.broadcasted_iota(jnp.int32, q.shape, 0) + lo // 2
        q = jnp.where((r >= DH * j // 2) & (r < DH * (j + 1) // 2), q, jnp.uint32(0))
        parts = [pltpu.bitcast(q, bf16)]
        if lo:
            parts.insert(0, jnp.zeros((lo, BQ), bf16))
        if hi < 128:
            parts.append(jnp.zeros((128 - hi, BQ), bf16))
        return jnp.concatenate(parts, axis=0)

    def qk_step(g, q, c, buf, m):
        s = _dot(kk[g, pl.ds(c * CK, CK), :], q)
        buf[pl.ds(c * CK, CK), :] = s
        mm = jnp.max(s.reshape(CK // 8, 8, BQ), axis=0)
        return mm if m is None else jnp.maximum(m, mm)

    def pv_step(h, c, buf, m, acc, zero):
        rows = pl.ds(pl.multiple_of(zero + c * CK, CK), CK)
        p = jnp.exp2(buf[rows, :] - m).astype(bf16)
        o = _dot(vt[h, :, pl.ds(c * CK, CK)], p)
        return o if acc is None else acc + o

    def finish(h, qb, j, acc):
        den = acc[DH:DH + 1] if j % 2 == 0 else acc[0:1]
        ot[pl.ds(pl.multiple_of(h * HP, HP), HP), pl.ds(pl.multiple_of(qb * BQ, BQ), BQ)] = (
            acc * (1.0 / den)).astype(bf16)

    def colmax(m):
        return jnp.max(m, axis=0, keepdims=True)

    def item(idx, j, m_prev, m_cur, acc, zero, do_qk=True, do_prev=True, do_cur=True):
        nxt = idx + 1
        if do_qk:
            gq = (nxt // G) % (H // G)
            q = load_q(gq, nxt // H, (j + 1) % G)
        mn = None
        for c in range(NC):
            if do_qk:
                mn = qk_step(gq, q, c, sbuf[(j + 1) % G], mn)
            cc = c - LAG
            if cc < 0:
                if do_prev:
                    acc = pv_step((idx - 1) % H, cc + NC, sbuf[(j - 1) % G], m_prev, acc, zero)
                    if cc == -1:
                        finish((idx - 1) % H, (idx - 1) // H, (j - 1) % G, acc)
                        acc = None
            elif do_cur:
                acc = pv_step(idx % H, cc, sbuf[j], m_cur, acc, zero)
        return m_cur, (colmax(mn) if do_qk else None), acc

    zero = pl.program_id(0) * CK
    n_items = H * NQ
    _, m, _ = item(-1, G - 1, None, None, None, zero, do_prev=False, do_cur=False)
    carry = item(0, 0, None, m, None, zero, do_prev=False)
    carry = item(1, 1, *carry, zero)
    carry = item(2, 2, *carry, zero)

    def body(it, carry):
        for u in range(G):
            carry = item(it * G + 3 + u, (3 + u) % G, *carry, zero)
        return carry

    carry = lax.fori_loop(0, n_items // G - 1, body, carry)
    carry = item(n_items - 1, G - 1, *carry, zero, do_qk=False)
    item(n_items, 0, *carry, zero, do_qk=False, do_cur=False)

    n2 = S // TN2
    o_cp = [pltpu.make_async_copy(yt.at[:, pl.ds(c * TN2, TN2)],
                                  out_hbm.at[:, pl.ds(c * TN2, TN2)], sem_o.at[c]) for c in range(n2)]
    ones_rows = jnp.where(lax.broadcasted_iota(jnp.int32, (KP - D, TN2), 0) == 0, 1.0, 0.0).astype(bf16)

    def proj(c):
        cols = pl.ds(c * TN2, TN2)
        h = xt[:, cols].astype(f32) + _dot(wot[...], ot[:, cols])
        s0[pl.ds(c * D, D), pl.ds(0, TN2)] = h
        return jnp.concatenate([_layernorm_t(h).astype(bf16), ones_rows], axis=0)

    ln = proj(0)
    for c in range(n2):
        cols = pl.ds(c * TN2, TN2)
        cur = ln
        if c + 1 < n2:
            ln = proj(c + 1)
        a = jnp.maximum(_dot(w1t[...], cur), 0.0)
        y = _dot(w2t[...], (a * a).astype(bf16))
        h = s0[pl.ds(pl.multiple_of(zero + c * D, 8), D), pl.ds(0, TN2)]
        yt[:, cols] = (y + h + jnp.tile(b2c[...], (1, TN2 // 128))).astype(yt.dtype)
        o_cp[c].start()
    for cp in o_cp:
        cp.wait()


def make(LAG=1, TN0=512, TN2=512, name="blk", flags=None):
    def fn(A_x, A_wqkv, A_wo, B_x, B_w1, B_b1, B_w2, B_b2):
        del B_x
        hbm = pl.BlockSpec(memory_space=pltpu.HBM)
        vm = lambda shape: pl.BlockSpec(shape, lambda i: (0,) * len(shape))
        out_t = pl.pallas_call(
            functools.partial(_kernel, LAG, TN0, TN2),
            grid=(1,),
            in_specs=[hbm, hbm, hbm, hbm, vm((1, F)), hbm, vm((1, D))],
            out_specs=hbm,
            out_shape=jax.ShapeDtypeStruct((D, S), A_x.dtype),
            scratch_shapes=[
                pltpu.VMEM((D, S), bf16),
                pltpu.VMEM((D, 3 * D), bf16),
                pltpu.VMEM((D, D), bf16),
                pltpu.VMEM((D, F), bf16),
                pltpu.VMEM((D, F), bf16),
                pltpu.VMEM((3 * D, D), bf16),
                pltpu.VMEM((D, KP), bf16),
                pltpu.VMEM((F, KP), bf16),
                pltpu.VMEM((D, 128), f32),
                pltpu.VMEM((D, S), bf16),
                pltpu.VMEM((H // G, S, 128), bf16),
                pltpu.VMEM((H, HP, S), bf16),
                pltpu.VMEM((H * HP, S), bf16),
                pltpu.VMEM((D, S), A_x.dtype),
                *[pltpu.VMEM((S, BQ), f32)] * G,
                pltpu.SemaphoreType.DMA((S // TN0,)),
                pltpu.SemaphoreType.DMA((4,)),
                pltpu.SemaphoreType.DMA((S // TN2,)),
            ],
            compiler_params=pltpu.CompilerParams(
                dimension_semantics=("arbitrary",), vmem_limit_bytes=100 * 2**20, flags=flags),
            name=name,
        )(A_x.reshape(S, D).T, A_wqkv, A_wo, B_w1, B_b1.reshape(1, F), B_w2.T, B_b2.reshape(1, D))
        return out_t.T.reshape(A_x.shape)
    return fn


@jax.jit
def pallas_sequential_preLN__softmax_full_mha__dense_activation_squared_relu__prompt_kernel(
    A_x, A_wqkv, A_wo, B_x, B_w1, B_b1, B_w2, B_b2
):
    return make()(A_x, A_wqkv, A_wo, B_x, B_w1, B_b1, B_w2, B_b2)
```

```python
import functools
import math

import jax
import jax.numpy as jnp
from jax import lax
import jax.experimental.pallas as pl
import jax.experimental.pallas.tpu as pltpu

S, D, H, F = 2048, 448, 16, 1792
DH = D // H
HP = 32
BQ = 512
CK = 128
NC = S // CK
NQ = S // BQ
T0 = 256
N0 = S // T0
FE = 1536
EPS = 1e-5
QSCALE = DH ** -0.5 * math.log2(math.e)

f32, bf16, u32 = jnp.float32, jnp.bfloat16, jnp.uint32


def _dot(a, b):
    return jnp.dot(a, b, preferred_element_type=f32)


def _put(ref, i, row, lane, x):
    ref.bitcast(bf16)[pl.ds(i, 1), pl.ds(row, x.shape[0]), pl.ds(lane, x.shape[1])] = x[None].astype(bf16)


def _unpack(x):
    return pltpu.bitcast(x, bf16)


def _pad_rows(x, n):
    return x if x.shape[0] == n else jnp.concatenate(
        [x, jnp.zeros((n - x.shape[0], x.shape[1]), x.dtype)], axis=0)


def _up(n, m):
    return -(-n // m) * m


_PRODUCTS = (
    (((1, 1, 1),), ((1, 1, 0), (-1, 0, 0))),
    (((1, 1, 0), (1, 1, 1)), ((1, 0, 0),)),
    (((1, 0, 0),), ((1, 0, 1), (-1, 1, 1))),
    (((1, 0, 0), (1, 0, 1)), ((1, 1, 1),)),
    (((1, 0, 0), (1, 1, 1)), ((1, 0, 0), (1, 1, 1))),
    (((1, 0, 1), (-1, 1, 1)), ((1, 1, 0), (1, 1, 1))),
    (((1, 1, 0), (-1, 0, 0)), ((1, 0, 0), (1, 0, 1))),
)
_RESULTS = {
    1: ((1, 0), ((1, 0),)),
    3: ((0, 1), ((1, 2),)),
    5: ((0, 0), ((1, 0), (-1, 3), (1, 4))),
    6: ((1, 1), ((1, 2), (-1, 1), (1, 4))),
}


def _signed_sum(terms):
    (_, v), *rest = terms
    for sign, w in rest:
        v = v.astype(f32) + w.astype(f32) if sign > 0 else v.astype(f32) - w.astype(f32)
    return v


def _operands(block, level, side):
    if level == 0:
        yield block(0, 0)
        return
    n = 2 ** (level - 1)
    for prod in _PRODUCTS:
        sub = {(i, j): _signed_sum([(sign, block(qi * n + i, qj * n + j)) for sign, qi, qj in prod[side]])
               for i in range(n) for j in range(n)}
        yield from _operands(lambda i, j: sub[i, j], level - 1, side)


def _quadrants(product):
    seen = []
    for p in range(7):
        seen.append(product(p))
        if p in _RESULTS:
            quadrant, earlier = _RESULTS[p]
            yield quadrant, _signed_sum([(sign, seen[e]) for sign, e in earlier] + [(1, seen[p])])


def _row_chunks(rows, size):
    n = -(-rows // size)
    edges = [16 * ((rows // 16 * i) // n) for i in range(n + 1)]
    return list(zip(edges[:-1], edges[1:]))


def _head_rows(a, h, fill):
    return jnp.concatenate(
        [a[DH * h:DH * (h + 1)], jnp.full((HP - DH, a.shape[1]), fill, a.dtype)], axis=0)


def _chain(*jobs):
    return (v for gen, _ in jobs for v in gen), sum(n for _, n in jobs)


def _share(job, parts):
    return [(job[0], job[1] * (i + 1) // parts - job[1] * i // parts) for i in range(parts)]


def _finish(job):
    for _ in job[0]:
        pass


def _spread(steps, *jobs):
    return ([v for gen, n in jobs for _ in range(n * (i + 1) // steps - n * i // steps) for v in next(gen)]
            for i in range(steps)), steps


def _kernel(cfg,
            xt_hbm, wqkv_hbm, wo_hbm, w1_hbm, b1_hbm, w2t_hbm, b2_hbm, out_hbm,
            xt, t1, ao, a2, a2l, b2c, qt, kk, vt, ot, last, acc, sem_in, sem_out):
    VK, HU, PH = cfg["VK"], cfg["HU"], cfg["PH"]
    ao, a2, a2l = (ao, D // 2, 256), (a2, D // 4, FE // 4), (a2l, D // 2, 128)
    zero = lax.fori_loop(0, 2, lambda i, z: z + (i >> 4), 0)
    zs = [zero >> i for i in range(8)]
    true = []
    first_vreg = lambda ref: [ref[zs[0], pl.ds(0, 8), pl.ds(0, 128)]]
    issued, held = [0], []

    def tie(x, job):
        n = min(x.shape[1], 128)
        tied = [pltpu.bitcast(v, u32)[:, :n] for v in next(job[0], [])]
        if not tied:
            return x
        lead = jnp.where(true[-1][:, :n], x[:, :n], functools.reduce(jnp.bitwise_or, tied))
        return jnp.concatenate([lead, x[:, n:]], axis=1) if x.shape[1] > n else lead

    def product(a_ops, b_ops, i, lo, hi, za, zb, job):
        (a_ref, _, k), (b_ref, rows, n) = a_ops, b_ops
        a = a_ref[za, pl.ds(lo // 2, (hi - lo) // 2), pl.ds(i * k, k)]
        a = [a[r:r + 8] for r in range(0, a.shape[0], 8)]
        r = issued[0] % 4 * len(a) // 4
        a[r] = tie(a[r], job)
        issued[0] += k * n // 128 ** 2
        b = _pad_rows(b_ref[zb, pl.ds(0, rows // 2), pl.ds(i * n, n)], k // 2)
        return _dot(_unpack(jnp.concatenate(a, axis=0)), _unpack(b))

    def matmul(a_ops, b_ops, use, size, side):
        chunks = _row_chunks(a_ops[1], size)
        job = _spread(7 * len(chunks) - cfg["ME"], *side)
        for t, (lo, hi) in enumerate(chunks):
            for quadrant, v in _quadrants(lambda p: product(a_ops, b_ops, p, lo, hi, zs[use % 8], zs[t % 8], job)):
                yield lo, quadrant, v

    def operands_job(dst, level, side, block, rows=None):
        dst, height, width = dst
        tiles = [(r, c) for r in rows or range(0, height, 16) for c in range(0, width, 128)]

        def run():
            for r, c in tiles:
                z = zs[0]
                load = functools.cache(lambda i, j: block(i, j, r, c, z))
                for p, v in enumerate(_operands(load, level, side)):
                    _put(dst, 0, r, p * width + c, v)
                    if p % 7 == 6:
                        z = zs[p // 7 + 1]
                        load.cache_clear()
                        yield first_vreg(dst)
        return run(), len(tiles) * 7 ** (level - 1)

    def transpose_job(dst, part):
        tiles = [(c, j) for c in range(0, 2 * dst.shape[1], 128) for j in range(dst.shape[0])]

        def run():
            for c, j in tiles:
                n = min(128, 2 * dst.shape[1] - c)
                dst[j, pl.ds(c // 2, n // 2), :] = pltpu.bitcast(_pad_rows(part(j, c, n), dst.shape[2]).astype(bf16).T, u32)
                yield first_vreg(dst)
        return _spread(len(tiles) * cfg["TW"] * dst.shape[2] // 128, (run(), len(tiles)))

    def weights_job(dst, turned, level, row):
        block = lambda i, j, r, c, z: _unpack(turned[z + j, pl.ds(row(i, r) // 2, 8), pl.ds(c, 128)])
        return operands_job(dst, level, 0, block)

    def layernorm_job(width, load):
        stat, step = [], 128 * 128 // width

        def moments():
            for p in range(2):
                total = None
                for r in range(0, D, step):
                    x = load(zs[7 - p], pl.ds(r, step), 0, width)
                    x = jnp.sum((jnp.square(x - stat[0]) if p else x).reshape(-1, 8, width), axis=0)
                    total = x if total is None else total + x
                    yield [total[:, c:c + 128] for c in range(0, width, 128)]
                stat.append(jnp.sum(total, axis=0, keepdims=True) * (1.0 / D))
            stat[1] = lax.rsqrt(stat[1] + EPS)
            yield []

        return (moments(), 2 * D // step + 1), lambda r, c, n: (
            load(zs[0], pl.ds(r, 16), c, n) - stat[0][:, c:c + n]) * stat[1][:, c:c + n]

    def pv(h, b, c, p, src, dst, job, risk, slot=None):
        v = [tie(vt[h, pl.ds(r, 8), pl.ds(c * CK, CK)], job) for r in (0, 8)]
        v = _unpack(jnp.concatenate(v, axis=0))
        o = lax.dot_general(v, p, (((1,), (0,)), ((), ())), preferred_element_type=f32)
        if c > 0:
            n = cfg["AR"] if src is not acc else 0
            o = o + jnp.concatenate(held[:1 if n else 0] + ([src[zs[0], pl.ds(n, HP - n)]] if n < HP else []), axis=0)
        if c < NC - 1:
            n = cfg["AR"] if dst is not acc else 0
            held[:] = [o[:n]] if n else []
            if n < HP:
                dst[0, pl.ds(n, HP - n)] = o[n:]
            return risk
        den = o[DH:DH + 1]
        inv = pltpu.reciprocal(den, approx=True)
        ot[b][h if slot is None else slot] = o * (inv * (2.0 - den * inv))
        return risk + (jnp.abs(jnp.sum(o.reshape(-1, 8, BQ), axis=0)) + (den + inv * 2.0 ** 80))

    def front(wqkv, wo, w1, w2t, tqkv, to, aqkv, r0, kt, kp, kb, qb, qw, state, q0, b1, b2):
        true.append(jnp.full((8, 128), zs[0]) == 0)
        aqkv, r0 = [(a, D // 2, 256) for a in aqkv], [(r, D // 2, 128) for r in r0]
        cols = lambda src, dst, lo, hi: (src.at[:, pl.ds(lo, hi - lo)], dst.at[0, :, pl.ds(lo, hi - lo)])
        xe = (0, T0, *cfg["XE"], S)
        copies = [pltpu.make_async_copy(src, dst, sem_in.at[i]) for i, (src, dst) in enumerate((
            cols(wqkv_hbm, wqkv, 384, 2 * D), *[cols(xt_hbm, xt, lo, hi) for lo, hi in zip(xe[:-1], xe[1:])],
            cols(wqkv_hbm, wqkv, 0, 384), cols(wqkv_hbm, wqkv, 2 * D, 3 * D),
            (w2t_hbm, w2t.at[0]), (wo_hbm, wo), (w1_hbm, w1), (b1_hbm, b1), (b2_hbm, b2)))]
        for cp in copies:
            cp.start()

        nv = VK // 16
        slab = [{16 * g % CK: g for g in range(nv) if (NC * g + cfg["SO"]) // nv == c} for c in range(NC)]
        SHIFT, PARK = HP, HP + 8

        def ln_job(c):
            stats, norm = layernorm_job(T0, lambda z, rows, lo, n: xt[z, rows, pl.ds(c * T0 + lo, n)].astype(f32))
            return _chain(stats, operands_job(r0[c], 1, 1, lambda i, j, r, *_: norm(i * D // 2 + r, 128 * j, 128)))

        def wqkv_job(p):
            lo = p * D // 128 * 128
            return (transpose_job(tqkv[p], lambda j, c, n: wqkv[0, pl.ds(j * D // 2, D // 2), pl.ds(lo + c, n)]),
                          weights_job(aqkv[p], tqkv[p], 1, lambda i, r: p * D - lo + i * D // 2 + r))

        def wo_part(j, c, n):
            w = wo[pl.ds(j * D // 2, D // 2), pl.ds(c, n)].astype(f32)
            return jnp.concatenate([_head_rows(w, h, 0.0) for h in range(H // 2)], axis=0)

        def w1_part(j, c, n):
            w = w1[pl.ds(j * D // 4, D // 4), pl.ds(c, n)]
            if j:
                return w
            row = lax.broadcasted_iota(jnp.int32, (16, n), 0)
            bias = b1[...].astype(f32).reshape(1, F)[:, c:c + n]
            return jnp.concatenate([w, jnp.where(row == 0, bias, 0.0).astype(bf16)], axis=0)

        def kb_job(h, dst):
            def run():
                for d in range(DH):
                    for lo in range(0, VK, 128):
                        n = min(128, VK - lo)
                        t = jnp.broadcast_to(kt[h, pl.ds(d, 1), pl.ds(lo, 128)], (128, 128))[:, :n].T
                        dst[pl.ds(lo // 16, n // 16), d] = t.reshape(n // 16, 16, 128)
                    yield [dst[zs[0], 0, pl.ds(0, 8)]]
            return run(), DH

        def turn_keys(h, dst):
            def run():
                for lo in range(0, S, 128):
                    dst[pl.ds(lo // 2, 64), :] = k = pltpu.bitcast(_unpack(kp[h, :, pl.ds(lo, 128)]).T, u32)
                    if lo % 512 == 384:
                        yield [jnp.concatenate([k[-8:], jnp.zeros((8, 128 - HP), u32)], axis=1)]
            return run(), S // 512

        def qb_job(h, b, dst, qt=qt):
            def run():
                for w in range(BQ // 128):
                    for d in range(DH):
                        if d % 8 == 0:
                            q = qt[h + zs[d // 8], pl.ds(d // 16 * 8, 8), pl.ds(b * BQ + w * 128, 128)]
                            q = _unpack(q).astype(f32)
                        dst[0, w // 2, d ^ 1, w % 2] = jnp.broadcast_to(q[d % 16:d % 16 + 1], (8, 128))
                        if d % 4 == 3:
                            yield [dst[zs[0], 0, 0, 0]] if d // 4 in cfg["QE"] else []
            return run(), BQ // 128 * DH // 4

        def vpu_job(h, b, table, rows, lazy, query, park):
            def run():
                for n, (w, g) in enumerate((w, g) for w in range(0, BQ, 256) for g in range(nv)):
                    for d in range(DH):
                        q = jnp.concatenate([rows[lazy[n % len(lazy)], w // 256, d ^ 1, i] for i in range(2)], axis=1)
                        t = jnp.tile(table[g, d], (1, 2)) * jnp.tile(q, (2, 1))
                        s = t if d == 0 else s + t
                    if g == 0:
                        shift = -24.0 - jnp.max(s, axis=0, keepdims=True)
                        top = pltpu.bitcast(shift, u32) & u32(0xFFFF0000)
                        low = pltpu.bitcast(shift - pltpu.bitcast(top, f32), u32) >> 16
                        park[0, pl.ds(SHIFT, 8), pl.ds(w, 256)] = jnp.broadcast_to(
                            pltpu.bitcast(top, f32) + pltpu.bitcast(low << 16, f32), (8, 256))
                        query[0, pl.ds(0, HP // 2), pl.ds(w, 256)] = pltpu.bitcast(qt[h, :, pl.ds(b * BQ + w, 256)], f32)
                        for i in (0, 128):
                            query[0, pl.ds(DH // 2, 1), pl.ds(w + i, 128)] = pltpu.bitcast(top + low, f32)[:, i:i + 128]
                    park[0, pl.ds(PARK + 16 * g, 16), pl.ds(w, 256)] = s
                    yield [park[zs[0], pl.ds(PARK, 8), pl.ds(0, 128)]]
            return run(), BQ // 256 * nv

        def project(p, c, side, fill):
            parts = {}
            for _, quadrant, v in matmul(aqkv[p], r0[c], c, cfg["RC0"], side):
                parts.setdefault(quadrant, []).append(v)
            for (i, j), v in parts.items():
                v = jnp.concatenate(v, axis=0)
                for h in range(H // 2):
                    yield i * H // 2 + h, c * T0 + j * 128, _head_rows(v, h, fill)

        ni = HU * NQ
        carried = state[ni]
        if "A" in PH:
            kt[...] = jnp.zeros(kt.shape, f32)
            last[...] = jnp.zeros(last.shape, f32)
            acc[...] = jnp.ones(acc.shape, f32)
            copies[0].wait()
            _finish(_chain(*wqkv_job(1)))
            copies[1].wait()
            _finish(ln_job(0))
            wv = wqkv_job(2)
            wq = wqkv_job(0)
            turns = _chain(wq[0], wv[0])
            wq = _share(_chain(_spread(cfg["A0"]), wq[1]), N0 - cfg["WW"])
            for c in range(N0):
                for i, e in enumerate(xe[1:-1], 2):
                    if (c + 1) * T0 == e:
                        copies[i].wait()
                if c == cfg["WW"]:
                    for cp in copies[len(xe):len(xe) + 2]:
                        cp.wait()
                    _finish(turns)
                side = [ln_job(c + 1)] if c + 1 < N0 else []
                side += [wq[c - cfg["WW"]]] if c >= cfg["WW"] else []
                for h, lo, k in project(1, c, side, 1.0):
                    for r, g in slab[lo // CK].items():
                        kt[h, :, pl.ds(16 * g, 16)] = k[:, r:r + 16]
                    _put(kp, h, 0, lo, k)
            view = kb.at[pl.ds(zs[1], HU + 1)]
            tables = [kb_job(zs[0] + h, view.at[h]) for h in range(HU + 1)]
            tile = lambda n, first, step: lambda i, j, r, c, z: w2t[
                z, pl.ds(i * D // n + r, 16), pl.ds(first + j * step + c, 128)]
            jobs = _chain(operands_job(a2, 2, 0, tile(4, 0, FE // 4)), operands_job(a2l, 1, 0, tile(2, FE, 128)),
                          qb_job(0, 0, qb[0], q0))
            for c, side in enumerate([wv[1], *_share(jobs, N0 - 1)]):
                if c == 1:
                    copies[-5].wait()
                    _finish(_chain(*tables[:cfg["NT"]]))
                for h, lo, q in project(0, c, [side], 0.0):
                    _put(qt, h, 0, lo, q * QSCALE)
                    if h == 0 and lo < BQ:
                        _put(q0, 0, 0, lo, q * QSCALE)
            for cp in copies[-4:]:
                cp.wait()
            _finish(_chain(transpose_job(to, wo_part), transpose_job(t1, w1_part), *tables[cfg["NT"]:],
                           *[turn_keys(zs[0] + h, kk.at[h]) for h in range(HU)]))
            b2c[0] = jnp.broadcast_to(b2[...].astype(f32).reshape(1, D), (128, D)).T
            lazy = [lax.rem(zero, 1025 + 2 * i) for i in range(2)] if cfg["AZ"] else zs[:4]
            jobs = _chain(_spread(cfg["A4"], vpu_job(zs[0], 0, view.at[0], qb[0], lazy, carried, carried)),
                          qb_job(0, 1, qb[1]), weights_job(ao, to, 1, lambda i, r: i * D // 2 + r))
            for c, side in enumerate(_share(jobs, N0)):
                for h, lo, v in project(2, c, [side], 1.0):
                    _put(vt, h, 0, lo, v)
        else:
            for cp in copies:
                cp.wait()

        def attend(it, carry):
            h0, (hm, risk) = it * HU, carry
            at = lambda i: (jnp.minimum(h0 + i // NQ, H - 1), i % NQ)
            hs = [lax.rem(h0, 1025 + 2 * i) for i in range(cfg["ZV"])]
            tables, keys = kb.at[pl.ds(hs[0], 2 * HU + 1)], kk.at[pl.ds(hm, 2 * HU)]
            turns = _chain(*[turn_keys(jnp.minimum(hm + u, H - 1), keys.at[u]) for u in range(HU, 2 * HU)])
            builds = [kb_job(jnp.minimum(hm + u + 1, H - 1), tables.at[u + 1]) for u in range(HU, 2 * HU)]
            builds = _spread(DH * HU, *builds) if cfg["KI"] else _chain(*builds)
            if cfg["KP"] == 3:
                _finish(turns)
                turns = _spread(1)
            later = _chain(_spread(2), *((turns, builds) if cfg["KP"] == 1 else (builds, turns)))
            if cfg["KP"]:
                later = _share(later, ni)
            else:
                _finish(later)
                later = [_spread(1) for _ in range(ni)]
            query = [carried, *qw, carried]
            job = _chain(_spread(cfg["LD"]), *[_spread(
                (S - VK) // 16 + 2 * NC - cfg["LE"],
                vpu_job(*at(i), tables.at[i // NQ], qb[i % ni], [x - h0 for x in hs], query[i], state[i]),
                _chain(qb_job(*at(i + 1), qb[(i + 1) % ni]), _spread(cfg["QS"])), later[i - 1]) for i in range(1, ni + 1)])
            due = jnp.maximum(hm - 1, 0), NQ - 1, NC - 1, last[zs[0]], acc, None
            for i in range(ni):
                for c in range(NC):
                    rows = [r for r in range(CK - 16, -1, -16) if r not in slab[c]]
                    k = [tie(keys[i // NQ, pl.ds((c * CK + r) // 2, 8), :], job) for r in rows]
                    s = _dot(_unpack(jnp.concatenate(k, axis=0)), _unpack(query[i][zs[c % 4], pl.ds(0, HP // 2)]))
                    park = state[i] if i else carried
                    parked = {r: park[zs[1], pl.ds(PARK + 16 * g, 16)] for r, g in slab[c].items()}
                    shift = park[zs[c % 4], pl.ds(SHIFT, 8)]
                    risk = pv(*due, job, risk)
                    if c < cfg["MT"] or i == 0 or cfg["AR"] == HP:
                        shift = jnp.where(jnp.tile(true[-1], (1, BQ // 128)), shift, s[:8])
                    p = {r: jnp.exp2(s[16 * n:16 * n + 16]) for n, r in enumerate(rows)}
                    p.update({r: jnp.exp2(v + jnp.tile(shift, (2, 1))) for r, v in parked.items()})
                    p = jnp.concatenate([p[r] for r in range(0, CK, 16)], axis=0)
                    due = hm + i // NQ, i % NQ, c, p if c % 4 < cfg["PF"] else p.astype(bf16), state[i], acc if (i, c) == (ni - 1, NC - 2) else state[i]
            _finish(job)
            last[0] = p
            return hm + HU, risk

        risk = jnp.zeros((8, BQ), f32)
        if "B" in PH:
            with jax.named_scope("loop"):
                _, risk = lax.fori_loop(0, H // HU, attend, (zero, risk))
        if PH != "ABC":
            def keep(i, c):
                v = ot[0][i][:16, :128] + ot[1][i][:16, :128] + ot[2][i][:16, :128] + ot[3][i][:16, :128] + risk[:1, :128]
                v += kb[i, 0, 0] + kt[i, :16, :128] + last[i >> 5, :16, :128] + acc[i >> 5, :16, :128] + qb[0][0, 0, i, 0][:1] + carried[i >> 5, :16, :128] + qb[1][0, 0, i, 0][:1] + b2c[i >> 5, :16]
                v += (qt[i][:, :128] + vt[i][:, :128] + kp[i][:, :128] + sum(x[i >> 5, :16, :128] for x in (ao[0], t1, a2[0], a2l[0]))).astype(f32)
                xt[0, pl.ds(0, 16), pl.ds(0, 128)] = v.astype(bf16)
                xt[0, pl.ds(16, 16), pl.ds(0, 32)] = _unpack(kk[i][200:208, :32])
                return c
            lax.fori_loop(0, H, keep, 0)
            pltpu.sync_copy(xt.at[0], out_hbm)
        acc[0, pl.ds(HP, 8)] = risk

    ops = lambda level, rows, lanes: pltpu.VMEM((1, _up(rows, 64) // 2, 7 ** level * lanes), u32)
    turned = lambda rows: pltpu.VMEM((2, rows // 2, 256), u32)
    pl.run_scoped(
        front,
        pltpu.VMEM((1, D, 3 * D), bf16), pltpu.VMEM((D, D), bf16), pltpu.VMEM((D, F), bf16), pltpu.VMEM((1, D, F), bf16),
        [turned(D), turned(D + 64), turned(D)], turned(D), [ops(1, D // 2, 256)] * 3, [ops(1, D // 2, 128)] * N0,
        pltpu.VMEM((H, HP, _up(VK, 128)), f32), pltpu.VMEM((H, HP // 2, S), u32),
        pltpu.VMEM((H + HU + 1, VK // 16, DH, 16, 128), f32),
        [pltpu.VMEM((1, BQ // 256, DH, 2, 8, 128), f32)] * (HU * NQ),
        [pltpu.VMEM((1, HP // 2, BQ), f32)] * (HU * NQ - 1),
        [pltpu.VMEM((1, HP + 8 + VK, BQ), f32)] * (HU * NQ + 1),
        pltpu.VMEM((1, HP // 2, BQ), u32), pltpu.VMEM((F,), bf16), pltpu.VMEM((D,), bf16))

    def exact_attention(i, _):
        h, b, n = i // NQ, i % NQ, S // 2

        def step(c, carry):
            m_old, o = carry
            s = _dot(_unpack(kk[h, pl.ds(pl.multiple_of(c * (n // 2), n // 2), n // 2), :]),
                     _unpack(qt[h, :, pl.ds(pl.multiple_of(b * BQ, BQ), BQ)]))
            m = jnp.maximum(m_old, jnp.max(s, axis=0, keepdims=True))
            new = _dot(_unpack(vt[h, :, pl.ds(pl.multiple_of(c * n, n), n)]), jnp.exp2(s - m).astype(bf16))
            return m, o * jnp.exp2(m_old - m) + new

        _, o = lax.fori_loop(0, S // n, step, (jnp.full((1, BQ), -jnp.inf, f32), jnp.zeros((HP, BQ), f32)))
        for j in range(NQ):
            @pl.when(b == j)
            def _():
                ot[j][h] = o / o[DH:DH + 1]

    def back(yt, a1, ro, r1, r2, r2l, parked, act, hres, h0, lnh):
        true.append(jnp.full((8, 128), zs[1]) == 0)
        a1, ro = (a1, F // 4, 128), [(r, H * HP // 2, 128) for r in ro]
        r1, r2, r2l = (r1, 128, 128), (r2, FE // 4, 128), (r2l, 128, 256)

        def o_job(c):
            return operands_job(ro[c], 1, 1, lambda i, j, r, _, z: ot[c * T0 // BQ][
                z + i * H // 2 + r // HP, pl.ds(r % HP, 16), pl.ds(c * T0 % BQ + j * 128, 128)])

        def ln_jobs(ref, b):
            stats, norm = layernorm_job(BQ, lambda z, rows, lo, n: ref[b + z, rows, pl.ds(lo, n)])

            def normalise():
                for r in range(0, D, 16):
                    lnh[0, pl.ds(r, 16)] = norm(r, 0, BQ)
                    yield first_vreg(lnh) if r % 32 else []

            block = lambda i, j, r, _, z: lnh[z, pl.ds(i * D // 4 + r, 16), pl.ds(128 * j, 128)]
            return stats, _chain((normalise(), D // 16), operands_job(r1, 2, 1, block, range(0, D // 4, 16)))

        def out_proj(carry):
            redo, _ = carry
            pl.when(redo > 0)(lambda: lax.fori_loop(0, H * NQ, exact_attention, None))
            total = pv(H - 1, NQ - 1, NC - 1, last[zs[0]], acc, None, _spread(1), acc[zs[0], pl.ds(HP, 8)], H - 1 + redo)
            unsafe = jnp.max(jnp.where(total < 2.0 ** 120, 0, 1))
            _finish(o_job(0))
            hidden = lambda i, r: i * FE // 4 + r if r < FE // 4 else FE + i * (F - FE) // 4 + r - FE // 4
            one = lambda i, *_: jnp.full((16, 128), float(i == 0), f32)
            w1_job = _chain(operands_job(r1, 2, 1, one, [D // 4]),
                            weights_job(a1, t1, 2, hidden))
            ln = [_spread(1), _spread(1), *_share(_chain(_spread(4), *ln_jobs(h0, 0)), N0 - 2)]
            for c, side in enumerate(zip(ln, _share(w1_job, N0))):
                side = [*side] + ([o_job(c + 1)] if c + 1 < N0 else [])
                for lo, (i, j), v in matmul(ao, ro[c], c, cfg["RCO"], side):
                    rows, at = pl.ds(i * D // 2 + lo, v.shape[0]), c * T0 + j * 128
                    hres[at // BQ, rows, pl.ds(at % BQ, 128)] = v = v + xt[0, rows, pl.ds(at, 128)].astype(f32)
                    if at < BQ:
                        h0[0, rows, pl.ds(at, 128)] = v
            return redo + 1, unsafe

        def outer_level(inner):
            for p in range(7):
                for (i, j), v in inner(p):
                    at = (pl.ds(0, v.shape[0]), pl.ds(128 * (2 * i + j), 128))
                    if p < len(parked):
                        parked[p][(0, *at)] = v
                    if p in _RESULTS:
                        (qi, qj), earlier = _RESULTS[p]
                        yield (2 * qi + i, 2 * qj + j), _signed_sum(
                            [(sign, parked[e][(zs[p], *at)]) for sign, e in earlier] + [(1, v)])

        def ffn(b, _):
            n = D // 64
            issued[0] = 0
            ln = ln_jobs(hres, jnp.minimum(b + 1, NQ - 1))
            load = lambda t, i, r, c, z: act[t % 3][z, i, pl.ds(r % 64, 16), pl.ds(c, 128)]
            jobs = [operands_job(r2, 2, 1, lambda i, j, r, _, z: load(r // 64, i, r, 128 * j, z),
                                 range(64 * t, 64 * t + 64, 16)) for t in range(n - 1)]
            late = operands_job(r2l, 1, 1, lambda i, j, r, c, z: load(n - 1, 2 * i + r // 64, r, 256 * j + c, z))
            job = _chain(_spread(4), _spread(45 + cfg["M0"], ln[0]), *[_spread(49, job) for job in jobs[:-1]],
                         _spread(49 - cfg["M0"] - cfg["M1"], jobs[-1]))
            for t in range(n):
                inner = lambda p: _quadrants(lambda q: product(a1, r1, 7 * p + q, 64 * t, 64 * t + 64, 0, zs[t], job))
                for (i, j), v in outer_level(inner):
                    act[t % 3][0, i, :, pl.ds(128 * j, 128)] = jnp.square(jnp.maximum(v, 0.0))
            chunks = _row_chunks(D // 4, cfg["RC2"])
            job = _spread(49 * len(chunks), _chain(_spread(6), late, ln[1]))
            for t, (lo, hi) in enumerate(chunks):
                inner = lambda p: _quadrants(lambda q: product(a2, r2, 7 * p + q, lo, hi, 0, zs[t], job))
                for (i, j), v in outer_level(inner):
                    rows, lanes = pl.ds(i * D // 4 + lo, hi - lo), pl.ds(128 * j, 128)
                    h0[0, rows, lanes] = v + (hres[b, rows, lanes] + b2c[zs[j], rows])
            sent = [0, 0]
            for lo, (i, j), v in matmul(a2l, r2l, 0, cfg["RCL"], []):
                rows, lanes, hi = pl.ds(i * D // 2 + lo, v.shape[0]), pl.ds(256 * j, 256), lo + v.shape[0]
                yt[b, rows, lanes] = (v + h0[zs[0], rows, lanes]).astype(yt.dtype)
                if i == j and hi >= cfg["OH"]:
                    rows, sent[i] = pl.ds(i * D // 2 + sent[i], hi - sent[i]), hi
                    pltpu.make_async_copy(
                        yt.at[b, rows], out_hbm.at[rows, pl.ds(pl.multiple_of(b * BQ, BQ), BQ)], sem_out).start()

        lax.while_loop(lambda carry: carry[0] <= carry[1], out_proj, (0, 0))
        with jax.named_scope("ffn"):
            lax.fori_loop(0, NQ, ffn, None)
        with jax.named_scope("owait"):
            pltpu.make_async_copy(yt, yt, sem_out).wait()

    if "C" in PH:
        pl.run_scoped(
            back,
            pltpu.VMEM((NQ, D, BQ), out_hbm.dtype), ops(2, F // 4, 128), [ops(1, 256, 128)] * N0,
            ops(2, 128, 128), ops(2, FE // 4, 128), ops(1, 128, 256),
            [pltpu.VMEM((1, 112, BQ), f32)] * 5, [pltpu.VMEM((1, 4, 64, BQ), f32)] * 3,
            pltpu.VMEM((NQ, D, BQ), f32), pltpu.VMEM((1, D, BQ), f32), pltpu.VMEM((1, D, BQ), f32))


def make(name="blk", flags=None, **kw):
    cfg = dict(RC0=48, RCO=48, RC2=64, RCL=48, ME=1, M0=12, M1=3, TW=3, OH=0, VK=240, HU=2, SO=0, LD=6, LE=0,
               QE=range(7), QS=2, MT=2, XE=(512, 1024), WW=5, KP=0, PF=2, AR=24, KI=0, KZ=0, A0=56, NT=2, A1=2, A2=200, A3=10, A4=150, AZ=1, PH="ABC", ZV=4)
    cfg.update(kw)

    def fn(A_x, A_wqkv, A_wo, B_x, B_w1, B_b1, B_w2, B_b2):
        del B_x
        hbm = pl.BlockSpec(memory_space=pltpu.HBM)
        ops = lambda level, rows, lanes: pltpu.VMEM((1, _up(rows, 64) // 2, 7 ** level * lanes), u32)
        out_t = pl.pallas_call(
            functools.partial(_kernel, cfg),
            in_specs=[hbm] * 7,
            out_specs=hbm,
            out_shape=jax.ShapeDtypeStruct((D, S), A_x.dtype),
            scratch_shapes=[
                pltpu.VMEM((1, D, S), bf16),
                pltpu.VMEM((4, F // 2, 128), u32),
                ops(1, D // 2, 256), ops(2, D // 4, FE // 4), ops(1, D // 2, 128),
                pltpu.VMEM((1, D, 128), f32),
                pltpu.VMEM((H, HP // 2, S), u32),
                pltpu.VMEM((H + cfg["HU"], S // 2, HP), u32),
                pltpu.VMEM((H, HP // 2, S), u32),
                [pltpu.VMEM((H + 1, HP, BQ), f32)] * NQ,
                pltpu.VMEM((1, CK, BQ), f32), pltpu.VMEM((1, HP + 8, BQ), f32),
                pltpu.SemaphoreType.DMA((12,)),
                pltpu.SemaphoreType.DMA(()),
            ],
            compiler_params=pltpu.CompilerParams(vmem_limit_bytes=126 * 2**20, flags=flags),
            name=name,
        )(A_x.reshape(S, D).T, A_wqkv, A_wo, B_w1, B_b1, B_w2.T, B_b2)
        return out_t.T.reshape(A_x.shape)
    return fn


@jax.jit
def pallas_sequential_preLN__softmax_full_mha__dense_activation_squared_relu__prompt_kernel(
    A_x, A_wqkv, A_wo, B_x, B_w1, B_b1, B_w2, B_b2
):
    return make()(A_x, A_wqkv, A_wo, B_x, B_w1, B_b1, B_w2, B_b2)
```

```python
import functools
import math

import jax
import jax.numpy as jnp
from jax import lax
import jax.experimental.pallas as pl
import jax.experimental.pallas.tpu as pltpu

S, D, H, F = 2048, 448, 16, 1792
DH = D // H
HP = 32
BQ = 512
NQ = S // BQ
CK = 128
NC = S // CK
LAG = 2
T0 = 256
N0 = S // T0
FE = 1536
EPS = 1e-5
QSCALE = DH ** -0.5 * math.log2(math.e)

f32, bf16, u32, i32, i8 = jnp.float32, jnp.bfloat16, jnp.uint32, jnp.int32, jnp.int8


def _dot(a, b):
    return jnp.dot(a, b, preferred_element_type=f32)


def _put(ref, i, row, lane, x, dtype=bf16):
    ref.bitcast(dtype)[pl.ds(i, 1), pl.ds(row, x.shape[0]), pl.ds(lane, x.shape[1])] = x[None].astype(dtype)


def _unpack(x):
    return pltpu.bitcast(x, bf16)


def _pad_rows(x, n, fill=0):
    return x if x.shape[0] == n else jnp.concatenate(
        [x, jnp.full((n - x.shape[0], x.shape[1]), fill, x.dtype)], axis=0)


def _row_chunks(rows, size):
    n = -(-rows // size)
    edges = [16 * ((rows // 16 * i) // n) for i in range(n + 1)]
    return list(zip(edges[:-1], edges[1:]))


def _transpose(dst, part):
    for j in range(dst.shape[0]):
        for c in range(0, 2 * dst.shape[1], 128):
            n = min(128, 2 * dst.shape[1] - c)
            w = _pad_rows(part(j, c, n), dst.shape[2]).astype(bf16)
            dst[j, pl.ds(c // 2, n // 2), :] = pltpu.bitcast(w.T, u32)


def _tile(ref, j, r, c):
    return _unpack(ref[j, pl.ds(r // 2, 8), pl.ds(c, 128)]).astype(f32)


def _reciprocal(x):
    r = pltpu.reciprocal(x, approx=True)
    return r * (2.0 - x * r)


def _nearest(x, unit):
    rounded = x + 1.5 * 2.0 ** 23 * unit
    return pltpu.bitcast(rounded, i32), x - (rounded - 1.5 * 2.0 ** 23 * unit)


def _normalise(o, risk):
    den = o[DH:DH + 1]
    inv = _reciprocal(den)
    risk += jnp.abs(jnp.sum(o.reshape(-1, 8, o.shape[1]), axis=0)) + (den + inv * 2.0 ** 80)
    return o * inv, risk


_PRODUCTS = (
    (((1, 1, 1),), ((1, 1, 0), (-1, 0, 0))),
    (((1, 1, 0), (1, 1, 1)), ((1, 0, 0),)),
    (((1, 0, 0),), ((1, 0, 1), (-1, 1, 1))),
    (((1, 0, 0), (1, 0, 1)), ((1, 1, 1),)),
    (((1, 0, 0), (1, 1, 1)), ((1, 0, 0), (1, 1, 1))),
    (((1, 0, 1), (-1, 1, 1)), ((1, 1, 0), (1, 1, 1))),
    (((1, 1, 0), (-1, 0, 0)), ((1, 0, 0), (1, 0, 1))),
)
_RESULTS = {
    1: ((1, 0), ((1, 0),)),
    3: ((0, 1), ((1, 2),)),
    5: ((0, 0), ((1, 0), (-1, 3), (1, 4))),
    6: ((1, 1), ((1, 2), (-1, 1), (1, 4))),
}
LEFT, RIGHT = 0, 1


def _signed_sum(terms):
    (_, v), *rest = terms
    for sign, w in rest:
        v = v + w if sign > 0 else v - w
    return v


def _quadrants(product):
    seen = []
    for p in range(7):
        seen.append(product(p))
        if p in _RESULTS:
            quadrant, earlier = _RESULTS[p]
            yield quadrant, _signed_sum([(sign, seen[e]) for sign, e in earlier] + [(1, seen[p])])


def _chain(*jobs):
    return (v for gen, _ in jobs for v in gen), sum(n for _, n in jobs)


def _spread(steps, *jobs):
    return ([v for gen, n in jobs for _ in range(n * (i + 1) // steps - n * i // steps) for v in next(gen)]
            for i in range(steps)), steps


def _share(job, parts):
    return [(job[0], job[1] * (i + 1) // parts - job[1] * i // parts) for i in range(parts)]


def _finish(job):
    for _ in job[0]:
        pass


class _Ops:
    def __init__(self):
        zero = lax.fori_loop(0, 2, lambda i, z: z + (i >> 4), 0)
        self.zs = [zero >> i for i in range(8)]
        self.true = jnp.full((8, 128), zero) == 0
        self.tiles, self.latest = 0, None

    def after(self, x):
        n = x.shape[0] // 8
        return lax.select(jnp.tile(self.true, (n, 1)), x, jnp.tile(self.latest[:8, :128], (n, 1)))

    def witness(self, ref, row=0, lane=0):
        return [ref[self.zs[0], pl.ds(row, 8), pl.ds(lane, 128)]]

    def product(self, left, p, right, q, lo, hi, za, zb, job):
        (a_ref, na, _), (b_ref, nb, k) = left, right
        rows = pl.ds(lo // 2, (hi - lo) // 2)
        a = [a_ref[za, rows, pl.ds(c, 128)] for c in range(128 * p, a_ref.shape[2], 128 * na)]
        b = [b_ref[zb, pl.ds(0, k // 2), pl.ds(c, 128)] for c in range(128 * q, b_ref.shape[2], 128 * nb)]
        done = [v if v.dtype == u32 else pltpu.bitcast(v, u32) for v in next(job[0], [])]
        if done:
            r = self.tiles % 4 * (rows.size // 8) // 4 * 8
            tied = lax.select(self.true, a[0][r:r + 8], functools.reduce(lax.bitwise_or, done))
            a[0] = jnp.concatenate(
                ([a[0][:r]] if r else []) + [tied] + ([a[0][r + 8:]] if r + 8 < rows.size else []), axis=0)
        self.tiles += len(a) * len(b)
        self.latest = _dot(_unpack(jnp.concatenate(a, axis=1)),
                           _unpack(_pad_rows(jnp.concatenate(b, axis=1), 64 * len(a))))
        return self.latest

    def matmul(self, left, right, za, size, jobs):
        chunks = _row_chunks(left[2], size)
        job = _spread(7 * len(chunks) - 1, *jobs)
        for t, (lo, hi) in enumerate(chunks):
            for quadrant, v in _quadrants(lambda p: self.product(left, p, right, p, lo, hi, za, self.zs[t], job)):
                yield lo, quadrant, v

    def operands(self, dst, side, block, rows=None, first=0):
        ref, count, height = dst
        tiles = [(r, c) for r in rows or range(0, height, 16) for c in range(0, ref.shape[2] // count, 128)]

        def run():
            for r, c in tiles:
                tile = functools.cache(lambda i, j: block(i, j, r, c))
                sums = [_signed_sum([(sign, tile(i, j)) for sign, i, j in prod[side]]) for prod in _PRODUCTS]
                _put(ref, 0, r, c * count + 128 * first, jnp.concatenate(sums, axis=1))
                yield self.witness(ref, r // 2, c * count + 128 * first)
        return run(), len(tiles)

    def outer_operand(self, p, side, block):
        return lambda i, j, r, c: _signed_sum(
            [(sign, block(2 * qi + i, 2 * qj + j, r, c, self.zs[p])) for sign, qi, qj in _PRODUCTS[p][side]])

    def operands2(self, dst, side, block, rows):
        return _chain(*[self.operands(dst, side, self.outer_operand(p, side, block), [r], 7 * p)
                        for r in rows for p in range(7)])

    def layernorm(self, width, load):
        stat, step = [], 128 * 128 // width

        def run():
            for p in range(2):
                total = None
                for r in range(0, D, step):
                    x = load(self.zs[7 - p], pl.ds(r, step), 0, width)
                    x = jnp.sum((jnp.square(x - stat[0]) if p else x).reshape(-1, 8, width), axis=0)
                    total = x if total is None else total + x
                    yield [total[:, c:c + 128] for c in range(0, width, 128)]
                stat.append(jnp.sum(total, axis=0, keepdims=True) * (1.0 / D))
            stat[1] = lax.rsqrt(stat[1] + EPS)
            yield []

        return (run(), 2 * D // step + 1), lambda r, c, n: (
            load(self.zs[0], pl.ds(r, 16), c, n) - stat[0][:, c:c + n]) * stat[1][:, c:c + n]


def _kernel(xt_hbm, wqkv_hbm, wo_hbm, w1_hbm, b1_hbm, w2t_hbm, b2_hbm, out_hbm,
            xt, wqkv, wo, w1, w2t, yt, wqkvt, wot, w1t, b2c, aqkv, ao, a1, a2, a2r, lnx, heads, lnh, hid, hidr,
            qt, kt, vt, ot, key_stat, factors, q8, k8, qs, ks, last_p, last_o,
            parked, act, resid, part, normed, b1, b2, sem_in, sem_out):
    cols = lambda src, dst, lo, hi: (src.at[:, pl.ds(lo, hi - lo)], dst.at[0, :, pl.ds(lo, hi - lo)])
    copies = [pltpu.make_async_copy(src, dst, sem_in.at[i]) for i, (src, dst) in enumerate((
        cols(xt_hbm, xt, 0, 256), cols(wqkv_hbm, wqkv, 384, 2 * D),
        cols(xt_hbm, xt, 256, 512), cols(xt_hbm, xt, 512, 1024), cols(xt_hbm, xt, 1024, 1536),
        cols(xt_hbm, xt, 1536, S), cols(wqkv_hbm, wqkv, 0, 384), cols(wqkv_hbm, wqkv, 2 * D, 3 * D),
        (wo_hbm, wo), (w1_hbm, w1), (b1_hbm, b1), (w2t_hbm, w2t.at[0]), (b2_hbm, b2)))]
    for cp in copies:
        cp.start()

    def wait(lo, hi):
        for cp in copies[lo:hi]:
            cp.wait()

    ops = _Ops()
    zs = ops.zs
    aqkv, ao, a2r = [(a, 7, D // 2) for a in aqkv], (ao, 7, D // 2), (a2r, 7, D // 2)
    a1, a2, lnh = (a1, 49, F // 4), (a2, 49, D // 4), (lnh, 49, 128)
    lnx, heads = [(r, 7, D // 2) for r in lnx], [(r, 7, H * HP // 2) for r in heads]
    hid, hidr = [(r, 7, FE // 4) for r in hid], (hidr, 7, 128)

    lanes = lambda x: jnp.broadcast_to(x, (HP, 128))

    def over_tokens(ref, h, each, merges):
        totals = None
        for lo in range(0, NC, 4):
            x = [each(ref[zs[0] + h, lo + c]) for c in range(4)]
            x[0] = ops.after(x[0])
            parts = [functools.reduce(merge, x) for merge in merges]
            totals = [merge(a, b) for merge, a, b in zip(merges, totals, parts)] if lo else parts
            if lo + 4 < NC:
                yield []
        return totals

    def key_stats(h):
        total, high, low = yield from over_tokens(kt, h, lambda x: x, (jnp.add, jnp.maximum, jnp.minimum))
        key_stat[h, 0] = lanes(jnp.sum(total, axis=1, keepdims=True) * (1.0 / S))
        key_stat[h, 1] = lanes(jnp.max(high, axis=1, keepdims=True) - jnp.min(low, axis=1, keepdims=True))
        yield []

    def balance(h):
        top, = yield from over_tokens(qt, h, jnp.abs, (jnp.maximum,))
        ratio = (lanes(jnp.max(top, axis=1, keepdims=True)) + 2.0 ** -60) * _reciprocal(key_stat[h, 1] + 2.0 ** -60)
        ratio = jnp.clip(ratio, 2.0 ** -100, 2.0 ** 100)
        factors[h > 0][h, 0] = lax.rsqrt(ratio)
        factors[h > 0][h, 1] = lax.rsqrt(ratio) * ratio
        yield []

    def limbs_job(h, at, factors):
        def scaled(x, top):
            scale = jnp.maximum(jnp.max(jnp.abs(x), axis=0, keepdims=True) * (1.0 / top), 2.0 ** -100)
            inv, halves = jnp.broadcast_to(_reciprocal(scale), (8, CK)), []
            for r in (0, HP // 2):
                yield []
                halves.append(x[r:r + HP // 2] * jnp.tile(ops.after(inv), (2, 1)))
            return jnp.concatenate(halves, axis=0), scale

        def run():
            for c in range(NC):
                g = h + zs[c % 4]
                y, scale = yield from scaled((kt[g, c] - key_stat[g, 0]) * ops.after(factors[g, 1]), 127)
                v, rest = _nearest(y, 1)
                limbs = [v, v, _nearest(rest, 1 / 16)[0], _nearest(y, 16)[0]]
                _put(k8[at], 0, 0, c * CK, jnp.concatenate(limbs, axis=0).T, i8)
                ks[at][0, pl.ds(c * CK, CK)] = jnp.broadcast_to(scale, (CK, CK)).T
                yield []
            for c in range(NC):
                g = h + zs[c % 4]
                x, scale = yield from scaled(qt[g, c] * ops.after(factors[g, 0]), 254)
                (u, rest), (u1, _) = _nearest(x, 1), _nearest(x, 2)
                limbs = [u1, u - u1, _nearest(x, 16)[0], _nearest(rest, 1 / 16)[0]]
                _put(q8[at], 0, 0, c * CK, jnp.concatenate(limbs, axis=0), i8)
                qs[at][0, :, pl.ds(c * CK, CK)] = jnp.broadcast_to(scale, (8, CK))
                yield []
        return run(), 6 * NC

    def ln_job(c):
        stats, norm = ops.layernorm(T0, lambda z, rows, lo, n: xt[z, rows, pl.ds(c * T0 + lo, n)].astype(f32))
        return _chain(stats, ops.operands(lnx[c], RIGHT, lambda i, j, r, _: norm(i * D // 2 + r, 128 * j, 128)))

    def weights_job(p):
        lo = p * D // 128 * 128
        _transpose(wqkvt[p], lambda j, c, n: wqkv[0, pl.ds(j * D // 2, D // 2), pl.ds(lo + c, n)])
        return ops.operands(
            aqkv[p], LEFT, lambda i, j, r, c: _tile(wqkvt[p], zs[0] + j, p * D - lo + i * D // 2 + r, c))

    def project(p, c, za, jobs, fill):
        parts = {}
        for _, quadrant, v in ops.matmul(aqkv[p], lnx[c], za, 48, jobs):
            parts.setdefault(quadrant, []).append(v)
        for (i, j), v in parts.items():
            v = jnp.concatenate(v, axis=0)
            for h in range(H // 2):
                yield i * H // 2 + h, 2 * c + j, _pad_rows(v[DH * h:DH * (h + 1)], HP, fill)

    def turn_later_weights():
        def wo_part(j, c, n):
            w = wo[pl.ds(j * D // 2, D // 2), pl.ds(c, n)].astype(f32)
            return jnp.concatenate([_pad_rows(w[DH * h:DH * (h + 1)], HP) for h in range(H // 2)], axis=0)

        def w1_part(j, c, n):
            w = w1[pl.ds(j * D // 4, D // 4), pl.ds(c, n)]
            return w if j else jnp.concatenate([w, bias[:, c:c + n]], axis=0)

        wait(8, 11)
        bias = jnp.where(lax.broadcasted_iota(i32, (16, F), 0) == 0, b1[...].astype(f32).reshape(1, F), 0.0).astype(bf16)
        _transpose(wot, wo_part)
        _transpose(w1t, w1_part)

    last_p[...] = jnp.zeros(last_p.shape, u32)
    last_o[...] = jnp.ones(last_o.shape, f32)
    _finish(ops.operands2(
        lnh, RIGHT, lambda i, *_: jnp.full((16, 128), float(i == 0), f32), [D // 4]))
    wait(0, 1)
    _finish(ln_job(0))
    wait(1, 2)
    wk = weights_job(1)
    for c in range(N0):
        wait(*{0: (2, 3), 1: (3, 4), 3: (4, 5), 5: (5, 8)}.get(c, (0, 0)))
        if c == 0:
            _finish(wk)
        if c == 5:
            wq, wv = _share(_chain(_spread(56), weights_job(0)), N0 - 5), weights_job(2)
        jobs = ([ln_job(c + 1)] if c + 1 < N0 else []) + ([wq[c - 5]] if c >= 5 else [])
        for h, t, k in project(1, c, zs[c] if c else 0, jobs, 0):
            kt[h, t] = k

    job = _spread(200, _chain(_spread(1), *[(key_stats(h), 4) for h in range(H)], _spread(6)), _chain(
        _spread(28), ops.operands(ao, LEFT, lambda i, j, r, c: _tile(wot, zs[0] + j, i * D // 2 + r, c))))
    for c, share in enumerate(_share(wv, 2) + _share(job, N0 - 2)):
        if c == 3:
            turn_later_weights()
        for h, t, q in project(0, c, zs[c], [share], 0):
            qt[h, t] = q * QSCALE

    wait(11, 13)
    b2c[0] = jnp.broadcast_to(b2[...].astype(f32).reshape(1, D), (128, D)).T
    w2 = lambda r, c, z: w2t[z, pl.ds(r, 16), pl.ds(c, 128)].astype(f32)
    weights = _chain(
        ops.operands2(a2, LEFT, lambda i, j, r, c, z: w2(i * D // 4 + r, j * FE // 4 + c, z), range(0, D // 4, 16)),
        ops.operands(a2r, LEFT, lambda i, j, r, c: w2(i * D // 2 + r, FE + j * 128, zs[0])))
    steps = [(balance(h), 4) for h in range(H)]
    limbs = _chain(*steps[:2], _spread(
        200, _chain(limbs_job(0, 0, factors[0]), _spread(1)), _chain(*steps[2:], _spread(16))))
    for c, shares in enumerate(zip(_share(weights, N0), _share(limbs, N0))):
        for h, t, v in project(2, c, zs[c], shares, 1):
            _put(vt, h, 0, t * CK, v)

    def attend(it, carry):
        h0, *risk = carry
        job = _chain(*[_chain(_spread(2 * NQ * NC - 3, limbs_job(
            jnp.minimum(2 * it + u, H - 1), u % 2, factors[1])), _spread(3)) for u in (1, 2)])

        def half(n):
            w, z = n * BQ // 2, zs[4 * n]
            own = pl.ds(w, BQ // 2)
            due = [(jnp.maximum(h0 - 1, 0), NQ - 1, NC - LAG + t, _unpack(last_p[zs[0] + t, :, own]))
                   for t in range(LAG)]
            cuts = [0, *range(2 - n, NC, 2), NC]
            for u, b in ((u, b) for u in range(2) for b in range(NQ)):
                queries = pl.ds(b * BQ + w, BQ // 2)
                for lo, hi in zip(cuts[:-1], cuts[1:]):
                    k = [k8[u][z, pl.ds(r, 8), pl.ds(c * CK, CK)] for c in range(lo, hi) for r in (24, 16, 8, 0)]
                    s = jnp.dot(pltpu.bitcast(jnp.concatenate(k, axis=0), i8),
                                pltpu.bitcast(q8[u][z, :, queries], i8), preferred_element_type=i32).astype(f32)
                    for c in range(lo, hi):
                        ops.latest = x = s[(c - lo) * CK:(c - lo + 1) * CK]
                        x = jnp.concatenate([x[r:r + 32] for r in (96, 64, 32, 0)], axis=0)
                        x = x * jnp.tile(ks[u][z, pl.ds(c * CK, CK)], (1, 2))
                        due.append((h0 + u, b, c, jnp.exp2(x * jnp.tile(qs[u][z, :, queries], (CK // 8, 1)))))
                        next(job[0])
                    yield 64 * (hi - lo)
                    if hi % 2 != n and (u, b) != (1, NQ - 1):
                        continue
                    o = last_o[zs[0], :, own]
                    while len(due) > LAG:
                        h, block, c, p = due.pop(0)
                        new = _dot(_unpack(vt[h, :, pl.ds(c * CK, CK)]), p.astype(bf16))
                        o = new + o if c else new
                        if c == NC - 1:
                            ot[block][h, :, own], risk[n] = _normalise(o, risk[n])
                        yield 32
                    if c < NC - 1:
                        last_o[0, :, own] = o
            for t in range(LAG):
                _put(last_p, t, 0, w, due[t][3])

        clocks = [[0, n, half(n)] for n in range(2)]
        while clocks:
            first = min(clocks)
            cycles = next(first[2], None)
            if cycles is None:
                clocks.remove(first)
            else:
                first[0] += cycles
        return h0 + 2, *risk

    _, *risk = lax.fori_loop(0, H // 2, attend, (zs[0], *[jnp.zeros((8, BQ // 2), f32)] * 2))

    def attend_with_true_max(i, _):
        h, b, n = i // NQ, i % NQ, S // 2

        def step(c, carry):
            m_old, o = carry
            k = jnp.concatenate([kt[h, c * (n // CK) + t] for t in range(n // CK)], axis=1)
            q = jnp.concatenate([qt[h, b * (BQ // CK) + t] for t in range(BQ // CK)], axis=1)
            s = _dot(k.astype(bf16).T, q.astype(bf16))
            m = jnp.maximum(m_old, jnp.max(s, axis=0, keepdims=True))
            new = _dot(_unpack(vt[h, :, pl.ds(pl.multiple_of(c * n, n), n)]), jnp.exp2(s - m).astype(bf16))
            return m, o * jnp.exp2(m_old - m) + new

        _, o = lax.fori_loop(0, S // n, step, (jnp.full((1, BQ), -jnp.inf, f32), jnp.zeros((HP, BQ), f32)))
        for j in range(NQ):
            @pl.when(b == j)
            def _():
                ot[j][h] = o / o[DH:DH + 1]

    def heads_job(c):
        return ops.operands(heads[c], RIGHT, lambda i, j, r, _: ot[c * T0 // BQ][
            zs[0] + i * H // 2 + r // HP, pl.ds(r % HP, 16), pl.ds(c * T0 % BQ + j * 128, 128)])

    def ln_jobs(ref, b):
        stats, norm = ops.layernorm(BQ, lambda z, rows, lo, n: ref[b + z, rows, pl.ds(lo, n)])

        def run():
            for r in range(0, D, 16):
                normed[0, pl.ds(r, 16)] = norm(r, 0, BQ)
                yield ops.witness(normed) if r % 32 else []

        block = lambda i, j, r, _, z: normed[z, pl.ds(i * D // 4 + r, 16), pl.ds(128 * j, 128)]
        return stats, _chain((run(), D // 16), ops.operands2(lnh, RIGHT, block, range(0, D // 4, 16)))

    def out_projection(carry):
        again, _ = carry
        pl.when(again > 0)(lambda: lax.fori_loop(0, H * NQ, attend_with_true_max, None))
        o = _dot(_unpack(vt[H - 1, :, pl.ds(S - LAG * CK, LAG * CK)]),
                 _unpack(last_p[...].reshape(LAG * CK // 2, BQ))) + last_o[0]
        ot[NQ - 1][H - 1 + again], total = _normalise(o, jnp.concatenate(risk, axis=1))
        unsafe = jnp.max(jnp.where(total < 2.0 ** 120, 0, 1))
        ops.tiles = 0
        _finish(heads_job(0))
        unit = lambda i, r: i * FE // 4 + r if r < FE // 4 else FE + i * (F - FE) // 4 + r - FE // 4
        up = ops.operands2(a1, LEFT, lambda i, j, r, c, z: _tile(w1t, z + j, unit(i, r), c), range(0, F // 4, 16))
        ln = [_spread(1), _spread(1), *_share(_chain(_spread(4), *ln_jobs(part, 0)), N0 - 2)]
        for c, jobs in enumerate(zip(ln, _share(up, N0))):
            jobs = [*jobs] + ([heads_job(c + 1)] if c + 1 < N0 else [])
            for lo, (i, j), v in ops.matmul(ao, heads[c], zs[c], 48, jobs):
                rows, at = pl.ds(i * D // 2 + lo, v.shape[0]), c * T0 + j * 128
                resid[at // BQ, rows, pl.ds(at % BQ, 128)] = v = v + xt[0, rows, pl.ds(at, 128)].astype(f32)
                if at < BQ:
                    part[0, rows, pl.ds(at, 128)] = v
        return again + 1, unsafe

    def two_levels(product):
        for p in range(7):
            for (i, j), v in _quadrants(lambda q: product(p, q)):
                at = pl.ds(0, v.shape[0]), pl.ds(128 * (2 * i + j), 128)
                if p < len(parked):
                    parked[p][(0, *at)] = v
                if p in _RESULTS:
                    (qi, qj), earlier = _RESULTS[p]
                    yield (2 * qi + i, 2 * qj + j), _signed_sum(
                        [(sign, parked[e][(zs[p], *at)]) for sign, e in earlier] + [(1, v)])

    def feed_forward(b, _):
        ops.tiles = 0
        stats, ln = ln_jobs(resid, jnp.minimum(b + 1, NQ - 1))
        load = lambda t, i, r, c, z: act[t][z, i, pl.ds(r % 64, 16), pl.ds(c, 128)]
        hid_job = lambda p, rows: ops.operands(
            hid[p], RIGHT, ops.outer_operand(p, RIGHT, lambda i, j, r, _, z: load(r // 64, i, r, 128 * j, z)), rows)
        rest = range(FE // 4 - 64, FE // 4, 16)
        job = _chain(_spread(4), _spread(58, stats), _spread(278, _chain(
            *[hid_job(p, [r]) for r in range(0, rest[0], 16) for p in range(7)], hid_job(0, rest))))
        for t in range(len(act)):
            for (i, j), v in two_levels(
                    lambda p, q: ops.product(a1, 7 * p + q, lnh, 7 * p + q, 64 * t, 64 * t + 64, 0, zs[t], job)):
                act[t][0, i, :, pl.ds(128 * j, 128)] = jnp.square(jnp.maximum(v, 0.0))
        ln = [_spread(20, share) for share in _share(ln, 4)]
        job = _chain(*[_chain(_spread(6, hid_job(p, rest)), _spread(1)) for p in range(1, 7)], _spread(56, _chain(
            ops.operands(hidr, RIGHT, lambda i, j, r, c: load(-1, 2 * i + r // 64, r, 256 * j + c, zs[0])),
            *ln[:2])))
        for t, (lo, hi) in enumerate(_row_chunks(D // 4, 64)[::-1]):
            for (i, j), v in two_levels(lambda p, q: ops.product(a2, 7 * p + q, hid[p], q, lo, hi, 0, zs[t], job)):
                rows, at = pl.ds(i * D // 4 + lo, hi - lo), pl.ds(128 * j, 128)
                part[0, rows, at] = v + (resid[b, rows, at] + b2c[zs[j], rows])
        sent = [0, 0]
        for lo, (i, j), v in ops.matmul(a2r, hidr, zs[0], 32, [_chain(*ln[2:])]):
            rows, at, hi = pl.ds(i * D // 2 + lo, v.shape[0]), pl.ds(256 * j, 256), lo + v.shape[0]
            yt[b, rows, at] = (v + part[zs[0], rows, at]).astype(yt.dtype)
            if i == j and hi >= 64:
                rows, sent[i] = pl.ds(i * D // 2 + sent[i], hi - sent[i]), hi
                pltpu.make_async_copy(
                    yt.at[b, rows], out_hbm.at[rows, pl.ds(pl.multiple_of(b * BQ, BQ), BQ)], sem_out).start()

    lax.while_loop(lambda carry: carry[0] <= carry[1], out_projection, (0, 0))
    lax.fori_loop(0, NQ, feed_forward, None)
    pltpu.make_async_copy(yt, yt, sem_out).wait()


@jax.jit
def pallas_sequential_preLN__softmax_full_mha__dense_activation_squared_relu__prompt_kernel(
    A_x: jax.Array,
    A_wqkv: jax.Array,
    A_wo: jax.Array,
    B_x: jax.Array,
    B_w1: jax.Array,
    B_b1: jax.Array,
    B_w2: jax.Array,
    B_b2: jax.Array,
):
    del B_x
    hbm, vmem = pl.BlockSpec(memory_space=pltpu.HBM), pltpu.VMEM
    turned = lambda rows: vmem((2, rows // 2, 256), u32)
    operands = lambda count, rows, lanes: vmem((1, -(-rows // 64) * 32, count * lanes), u32)
    out_t = pl.pallas_call(
        _kernel,
        in_specs=[hbm] * 7,
        out_specs=hbm,
        out_shape=jax.ShapeDtypeStruct((D, S), A_x.dtype),
        scratch_shapes=[
            vmem((1, D, S), bf16),
            vmem((1, D, 3 * D), bf16),
            vmem((D, D), bf16),
            vmem((D, F), bf16),
            vmem((1, D, F), bf16),
            vmem((NQ, D, BQ), A_x.dtype),
            [turned(D), turned(D + 64), turned(D)],
            turned(D),
            vmem((4, F // 2, 128), u32),
            vmem((1, D, 128), f32),
            [operands(7, D // 2, 256)] * 3,
            operands(7, D // 2, 256),
            operands(49, F // 4, 128),
            operands(49, D // 4, FE // 4),
            operands(7, D // 2, 128),
            [operands(7, D // 2, 128)] * N0,
            [operands(7, H * HP // 2, 128)] * N0,
            operands(49, 128, 128),
            [operands(7, FE // 4, 128)] * 7,
            operands(7, 128, 256),
            vmem((H, NC, HP, CK), f32),
            vmem((H, NC, HP, CK), f32),
            vmem((H, HP // 2, S), u32),
            [vmem((H + 1, HP, BQ), f32)] * NQ,
            vmem((H, 2, HP, 128), f32),
            [vmem((n, 2, HP, 128), f32) for n in (1, H)],
            [vmem((1, HP, S), u32)] * 2,
            [vmem((1, CK // 4, S + CK), u32)] * 2,
            [vmem((1, 8, S), f32)] * 2,
            [vmem((1, S, CK), f32)] * 2,
            vmem((LAG, CK // 2, BQ), u32),
            vmem((1, HP, BQ), f32),
            [vmem((1, 64, BQ), f32)] * 5,
            [vmem((1, 4, 64, BQ), f32)] * (F // 256),
            vmem((NQ, D, BQ), f32),
            vmem((1, D, BQ), f32),
            vmem((1, D, BQ), f32),
            vmem((F,), bf16),
            vmem((D,), bf16),
            pltpu.SemaphoreType.DMA((13,)),
            pltpu.SemaphoreType.DMA(()),
        ],
        compiler_params=pltpu.CompilerParams(vmem_limit_bytes=100 * 2**20),
    )(A_x.reshape(S, D).T, A_wqkv, A_wo, B_w1, B_b1, B_w2.T, B_b2)
    return out_t.T.reshape(A_x.shape)
```
